```python
import os as _os
_os.environ.setdefault('JAX_PLATFORMS', 'cpu')
import jax
import jax.numpy as jnp

def _softmax(x, axis=-1):
    return jax.nn.softmax(x, axis=axis)

def _gelu(x):
    return jax.nn.gelu(x, approximate=True)

def _silu(x):
    return jax.nn.silu(x)

def _sigmoid(x):
    return jax.nn.sigmoid(x)

def _layernorm(x, axis=-1, eps=1e-05):
    m = jnp.mean(x, axis=axis, keepdims=True)
    v = jnp.var(x, axis=axis, keepdims=True)
    return (x - m) / jnp.sqrt(v + eps)

def _scatter_add(tgt, idx, src, axis=0):
    return tgt.at[idx].add(src)

def _segment_sum(src, seg, n):
    return jax.ops.segment_sum(src, seg, n)

class _Rng:

    def __init__(self, key):
        self._k = key

    def _next(self):
        self._k, sub = jax.random.split(self._k)
        return sub

    def normal(self, shape):
        return jax.random.normal(self._next(), shape, dtype=jnp.bfloat16)

    def randint(self, lo, hi, shape):
        return jax.random.randint(self._next(), shape, lo, hi, dtype=jnp.int32)

    def uniform(self, shape, lo=0.0, hi=1.0):
        return jax.random.uniform(self._next(), shape, jnp.bfloat16, lo, hi)

    def permutation(self, n):
        return jax.random.permutation(self._next(), n)
kernel_name = 'adaLN_cond__softmax_full_mha__mixer_gmlp__prompt'

def setup_inputs():
    _rng = _Rng(jax.random.key(int.from_bytes(__import__("os").urandom(4), "little")))
    _w = lambda a: (lambda t: t.astype(jnp.bfloat16) if jnp.issubdtype(t.dtype, jnp.floating) else t)(jnp.asarray(a))

    def _A_setup():
        B, S, D = (1, 2048, 512)
        return {'x': _w((lambda *s: _rng.normal(s) * 0.05)(B, S, D)), 'wqkv': _w((lambda *s: _rng.normal(s) * 0.05)(D, 3 * D)), 'wo': _w((lambda *s: _rng.normal(s) * 0.05)(D, D))}
    _A_in = _A_setup()

    def _B_setup():
        B, S, D, F = (1, 2048, 512, 1792)
        Fh = F // 2
        return {'x': _w((lambda *s: _rng.normal(s) * 0.05)(B, S, D)), 'w_in': _w((lambda *s: _rng.normal(s) * 0.4)(D, 2 * Fh)), 'w_sp': _w(0.01 * (lambda *s: _rng.normal(s) * 0.4)(S, S)), 'b_sp': _w(1.0 + 0.01 * (lambda *s: _rng.normal(s) * 0.05)(S)), 'w_out': _w((lambda *s: _rng.normal(s) * 0.05)(Fh, D))}
    _B_in = _B_setup()
    return {'A_x': _A_in['x'], 'A_wqkv': _A_in['wqkv'], 'A_wo': _A_in['wo'], 'B_x': _B_in['x'], 'B_w_in': _B_in['w_in'], 'B_w_sp': _B_in['w_sp'], 'B_b_sp': _B_in['b_sp'], 'B_w_out': _B_in['w_out'], 'c': _w((lambda *s: _rng.normal(s) * 0.05)(1, 512) * 8.0), 'w_mod': _w((lambda *s: _rng.normal(s) * 0.05)(512, 6 * 512) * 512 ** (-0.5) * 8.0)}

def reference(A_x, A_wqkv, A_wo, B_x, B_w_in, B_w_sp, B_b_sp, B_w_out, c, w_mod):

    def _A_ref(x, wqkv, wo):
        B, S, D = x.shape
        H = 32
        Dh = D // H
        qkv = (lambda x, *d: x.transpose(*d))((x @ wqkv).reshape(B, S, 3, H, Dh), 2, 0, 3, 1, 4)
        q, k, v = (qkv[0], qkv[1], qkv[2])
        scale = Dh ** (-0.5)
        scores = jnp.einsum('bhqd,bhkd->bhqk', q, k) * scale
        p = _softmax(scores, axis=-1)
        o = jnp.einsum('bhqk,bhkd->bhqd', p, v)
        return (lambda x, *d: x.transpose(*d))(o, 0, 2, 1, 3).reshape(B, S, D) @ wo

    def _B_ref(x, w_in, w_sp, b_sp, w_out):
        B, S, D = x.shape
        F = w_in.shape[-1]
        Fh = F // 2
        z = _gelu(jnp.einsum('bsd,df->bsf', x, w_in))
        z1 = z[..., :Fh].copy()
        z2 = _layernorm(z[..., Fh:], axis=-1)
        g = jnp.einsum('ts,bsf->btf', w_sp, z2) + b_sp[None, :, None]
        return jnp.einsum('bsf,fd->bsd', z1 * g, w_out)
    x = A_x
    mod = (_silu(c) @ w_mod).reshape(c.shape[0], 6, 1, -1)
    sa, ca, ga, sb, cb, gb = (mod[:, 0].copy(), mod[:, 1].copy(), mod[:, 2].copy(), mod[:, 3].copy(), mod[:, 4].copy(), mod[:, 5].copy())
    h = _layernorm(x, axis=-1) * (1 + ca) + sa
    x = x + ga * _A_ref(h, A_wqkv, A_wo)
    h = _layernorm(x, axis=-1) * (1 + cb) + sb
    x = x + gb * _B_ref(h, B_w_in, B_w_sp, B_b_sp, B_w_out)
    return x
```

```python
import functools
import math

import jax
import jax.numpy as jnp
from jax import lax
import jax.experimental.pallas as pl
import jax.experimental.pallas.tpu as pltpu

F32 = jnp.float32
BF16 = jnp.bfloat16

H = 32
EPS = 1e-5
TQ = 512
KC = 256
UPB = 4
TM = 256

L_LO = 2.0 ** -32
L_HI = 2.0 ** 64
F32_BIG = 3.0e38


def _layernorm(x):
    m = jnp.mean(x, axis=-1, keepdims=True)
    xc = x - m
    v = jnp.mean(xc * xc, axis=-1, keepdims=True)
    return xc * lax.rsqrt(v + EPS)


def _gelu(x):
    c = math.sqrt(2.0 / math.pi)
    return 0.5 * x * (1.0 + jnp.tanh(x * (c + (c * 0.044715) * (x * x))))


def _kernel(x_hbm, wqkv_hbm, wo_hbm, win_hbm, wsp_hbm, bsp_ref, wout_hbm, c_ref, wmod_hbm,
            out_hbm,
            x_v, wqkv_v, wo_v, win_v, wsp_v, wout_v, wmod_v,
            wqvt_v, mod_v, k_v, qt_v, vt_v, ot_v, x1_v, z1_v, z2_v, bcol_v, obuf,
            sems, osems, *, S, D, FH):
    DH = D // H
    NQ = S // TQ
    NKC = S // KC
    NU = H * NQ
    NB = S // TM
    HPG = 128 // DH

    cp_mod = pltpu.make_async_copy(wmod_hbm, wmod_v, sems.at[0])
    cp_x = pltpu.make_async_copy(x_hbm, x_v, sems.at[1])
    cp_qkv = pltpu.make_async_copy(wqkv_hbm, wqkv_v, sems.at[2])
    cp_wo = pltpu.make_async_copy(wo_hbm, wo_v, sems.at[3])
    cp_win = pltpu.make_async_copy(win_hbm, win_v, sems.at[4])
    cp_wsp = pltpu.make_async_copy(wsp_hbm, wsp_v, sems.at[5])
    cp_wout = pltpu.make_async_copy(wout_hbm, wout_v, sems.at[6])
    cp_qkv.start()
    cp_mod.start()
    cp_x.start()

    bcol_v[...] = jnp.transpose(jnp.broadcast_to(bsp_ref[...].astype(F32), (128, S)))

    cp_qkv.wait()
    wqvt_v[0:D, :] = jnp.transpose(wqkv_v[:, 0:D].astype(F32)).astype(BF16)
    wqvt_v[D:2 * D, :] = jnp.transpose(wqkv_v[:, 2 * D:3 * D].astype(F32)).astype(BF16)

    cp_mod.wait()
    cf = c_ref[...].astype(F32)
    sc = (cf * (1.0 / (1.0 + jnp.exp(-cf)))).astype(BF16)
    mod_v[...] = jnp.dot(jnp.broadcast_to(sc, (8, D)), wmod_v[...], preferred_element_type=F32)

    def modrow(i):
        return mod_v[0:1, i * D:(i + 1) * D]

    cp_x.wait()
    cp_wo.start()
    cp_win.start()
    cp_wsp.start()
    cp_wout.start()

    qscale = (DH ** -0.5) * math.log2(math.e)

    def p1_body(i, carry):
        r0 = pl.multiple_of(i * TM, TM)
        x = x_v[pl.ds(r0, TM), :].astype(F32)
        h = (_layernorm(x) * (1.0 + modrow(1)) + modrow(0)).astype(BF16)
        k = jnp.dot(h, wqkv_v[:, D:2 * D], preferred_element_type=F32).astype(BF16)
        for g in range(D // 128):
            k_v[g, pl.ds(r0, TM), :] = k[:, g * 128:(g + 1) * 128]
        qvt = lax.dot_general(wqvt_v[...], h, (((1,), (1,)), ((), ())),
                              preferred_element_type=F32)
        qt_v[:, pl.ds(r0, TM)] = (qvt[0:D] * qscale).astype(BF16)
        vt_v[:, pl.ds(r0, TM)] = qvt[D:2 * D].astype(BF16)
        return carry

    lax.fori_loop(0, NB, p1_body, 0)

    def wq_masked(u):
        h = u // NQ
        qb = u % NQ
        q = qt_v[pl.ds(pl.multiple_of(h * DH, DH), DH), pl.ds(pl.multiple_of(qb * TQ, TQ), TQ)]
        qrep = jnp.concatenate([q] * HPG, axis=0)
        rows = lax.broadcasted_iota(jnp.int32, (128, TQ), 0)
        return jnp.where((rows // DH) == (h % HPG), qrep, jnp.zeros_like(qrep))

    def qk(u, kc, wq):
        g = (u // NQ) // HPG
        return jnp.dot(k_v[g, pl.ds(kc * KC, KC), :], wq, preferred_element_type=F32)

    def pv(u, kc, p):
        h = u // NQ
        vt = vt_v[pl.ds(pl.multiple_of(h * DH, DH), DH), pl.ds(kc * KC, KC)]
        return jnp.dot(vt, p.astype(BF16), preferred_element_type=F32)

    def red(x, op):
        return op(x.reshape(KC // 8, 8, TQ), axis=0)

    def store_o(u, acc, lsum):
        h = u // NQ
        qb = u % NQ
        ot_v[pl.ds(pl.multiple_of(h * DH, DH), DH),
             pl.ds(pl.multiple_of(qb * TQ, TQ), TQ)] = acc * (1.0 / lsum)

    def fast_body(i, bad):
        n = UPB * NKC
        wqs, ss, st = {}, {}, {}
        for idx in range(n + 1):
            if idx < n:
                uu, kc = divmod(idx, NKC)
                u = i * UPB + uu
                if kc == 0:
                    wqs[uu] = wq_masked(u)
                ss[idx] = qk(u, kc, wqs[uu])
            if idx >= 1:
                uu, kc = divmod(idx - 1, NKC)
                u = i * UPB + uu
                p = jnp.exp2(ss.pop(idx - 1))
                a = pv(u, kc, p)
                r = red(p, jnp.sum)
                st[uu] = (a, r) if kc == 0 else (st[uu][0] + a, st[uu][1] + r)
                if kc == NKC - 1:
                    acc, l = st.pop(uu)
                    lsum = jnp.sum(l, axis=0, keepdims=True)
                    ok = jnp.logical_and(
                        jnp.logical_and(lsum >= L_LO, lsum <= L_HI),
                        jnp.abs(acc) <= F32_BIG)
                    bad = jnp.where(ok, bad, 1.0)
                    store_o(u, acc, lsum)
        return bad

    bad = lax.fori_loop(0, NU // UPB, fast_body, jnp.zeros((DH, TQ), F32))
    any_bad = jnp.max(bad) > 0.0

    @pl.when(any_bad)
    def _():
        def safe_body(u, carry):
            wq = wq_masked(u)
            acc = l = m = None
            for kc in range(NKC):
                s = qk(u, kc, wq)
                mc = jnp.max(red(s, jnp.max), axis=0, keepdims=True)
                if kc == 0:
                    m = mc
                    p = jnp.exp2(s - m)
                    acc = pv(u, kc, p)
                    l = red(p, jnp.sum)
                else:
                    mn = jnp.maximum(m, mc)
                    al = jnp.exp2(m - mn)
                    p = jnp.exp2(s - mn)
                    acc = acc * al + pv(u, kc, p)
                    l = l * al + red(p, jnp.sum)
                    m = mn
            store_o(u, acc, jnp.sum(l, axis=0, keepdims=True))
            return carry

        lax.fori_loop(0, NU, safe_body, 0)

    cp_wo.wait()
    cp_win.wait()

    def p3_body(i, carry):
        r0 = pl.multiple_of(i * TM, TM)
        o = jnp.transpose(ot_v[:, pl.ds(r0, TM)]).astype(BF16)
        a = jnp.dot(o, wo_v[...], preferred_element_type=F32)
        x1 = x_v[pl.ds(r0, TM), :].astype(F32) + modrow(2) * a
        x1_v[pl.ds(r0, TM), :] = x1
        h2 = (_layernorm(x1) * (1.0 + modrow(4)) + modrow(3)).astype(BF16)
        z1 = _gelu(jnp.dot(h2, win_v[:, 0:FH], preferred_element_type=F32))
        z1_v[pl.ds(r0, TM), :] = z1
        z2 = _gelu(jnp.dot(h2, win_v[:, FH:2 * FH], preferred_element_type=F32))
        z2_v[pl.ds(r0, TM), :] = _layernorm(z2).astype(BF16)
        return carry

    lax.fori_loop(0, NB, p3_body, 0)

    cp_wsp.wait()
    cp_wout.wait()

    def out_copy(i, slot):
        return pltpu.make_async_copy(
            obuf.at[slot], out_hbm.at[pl.ds(pl.multiple_of(i * TM, TM), TM), :], osems.at[slot])

    def p4_body(i, carry):
        r0 = pl.multiple_of(i * TM, TM)
        slot = i % 2
        g = jnp.dot(wsp_v[pl.ds(r0, TM), :], z2_v[...], preferred_element_type=F32)
        b = bcol_v[pl.ds(r0, TM), :]
        g = g + jnp.concatenate([b] * (FH // 128), axis=1)
        t = (z1_v[pl.ds(r0, TM), :] * g).astype(BF16)
        y = jnp.dot(t, wout_v[...], preferred_element_type=F32)
        res = (x1_v[pl.ds(r0, TM), :] + modrow(5) * y).astype(BF16)

        @pl.when(i >= 2)
        def _():
            out_copy(i - 2, slot).wait()

        obuf[slot] = res
        out_copy(i, slot).start()
        return carry

    lax.fori_loop(0, NB, p4_body, 0)
    out_copy(NB - 2, NB % 2).wait()
    out_copy(NB - 1, (NB - 1) % 2).wait()


@jax.jit
def pallas_adaLN_cond__softmax_full_mha__mixer_gmlp__prompt_kernel(
    A_x: jax.Array,
    A_wqkv: jax.Array,
    A_wo: jax.Array,
    B_x: jax.Array,
    B_w_in: jax.Array,
    B_w_sp: jax.Array,
    B_b_sp: jax.Array,
    B_w_out: jax.Array,
    c: jax.Array,
    w_mod: jax.Array,
):
    B, S, D = A_x.shape
    assert B == 1
    F = B_w_in.shape[-1]
    FH = F // 2
    any_spec = pl.BlockSpec(memory_space=pl.ANY)
    vmem_spec = pl.BlockSpec(memory_space=pltpu.VMEM)
    out = pl.pallas_call(
        functools.partial(_kernel, S=S, D=D, FH=FH),
        out_shape=jax.ShapeDtypeStruct((S, D), BF16),
        in_specs=[any_spec, any_spec, any_spec, any_spec, any_spec, vmem_spec,
                  any_spec, vmem_spec, any_spec],
        out_specs=any_spec,
        scratch_shapes=[
            pltpu.VMEM((S, D), BF16),
            pltpu.VMEM((D, 3 * D), BF16),
            pltpu.VMEM((D, D), BF16),
            pltpu.VMEM((D, F), BF16),
            pltpu.VMEM((S, S), BF16),
            pltpu.VMEM((FH, D), BF16),
            pltpu.VMEM((D, 6 * D), BF16),
            pltpu.VMEM((2 * D, D), BF16),
            pltpu.VMEM((8, 6 * D), F32),
            pltpu.VMEM((D // 128, S, 128), BF16),
            pltpu.VMEM((D, S), BF16),
            pltpu.VMEM((D, S), BF16),
            pltpu.VMEM((D, S), F32),
            pltpu.VMEM((S, D), F32),
            pltpu.VMEM((S, FH), F32),
            pltpu.VMEM((S, FH), BF16),
            pltpu.VMEM((S, 128), F32),
            pltpu.VMEM((2, TM, D), BF16),
            pltpu.SemaphoreType.DMA((7,)),
            pltpu.SemaphoreType.DMA((2,)),
        ],
        compiler_params=pltpu.CompilerParams(vmem_limit_bytes=100 * 1024 * 1024),
    )(A_x.reshape(S, D), A_wqkv, A_wo, B_w_in, B_w_sp, B_b_sp.reshape(1, S), B_w_out, c, w_mod)
    return out.reshape(B, S, D)
```

```python
import functools
import math
import os

import jax
import jax.numpy as jnp
from jax import lax
import jax.experimental.pallas as pl
import jax.experimental.pallas.tpu as pltpu

F32 = jnp.float32
BF16 = jnp.bfloat16

def _env(name, default):
    return int(os.environ.get(name, default))

H = 32
EPS = 1e-5
TQ = 512
KC = 256
UPB = _env("UPB", 8)
TM1 = _env("TM1", 256)
U1 = _env("U1", 8)
TM3 = _env("TM3", 256)
U3 = _env("U3", 1)
FAKE3 = _env("FAKE3", 0)
ACC0 = _env("ACC0", 0)
KV = 256
SB = 32
LAG = _env("LAG", 2)
KBDL = _env("KBDL", 56)
QVW = _env("QVW", 128)
NCH = _env("NCH", 3)
PVA = _env("PVA", 0)
PVB = _env("PVB", 2)
HPB = 2
TM4 = _env("TM4", 256)
U4 = _env("U4", 1)
FORCE_SAFE = _env("FORCE_SAFE", 0)
LATE_DMA = _env("LATE_DMA", 1)
P3ALT = _env("P3ALT", 1)

L_LO = 2.0 ** -32
L_HI = 2.0 ** 64
F32_BIG = 3.0e38


def _layernorm(x):
    m = jnp.mean(x, axis=-1, keepdims=True)
    xc = x - m
    v = jnp.mean(xc * xc, axis=-1, keepdims=True)
    return xc * lax.rsqrt(v + EPS)


def _gelu(x):
    c = math.sqrt(2.0 / math.pi)
    return 0.5 * x * (1.0 + jnp.tanh(x * (c + (c * 0.044715) * (x * x))))


def _loop(n, unroll, body):
    if unroll >= n:
        body([i for i in range(n)])
    else:
        def f(j, c):
            body([j * unroll + t for t in range(unroll)])
            return c
        lax.fori_loop(0, n // unroll, f, 0)


def _rows(i, tm):
    if isinstance(i, int):
        return pl.ds(i * tm, tm)
    return pl.ds(pl.multiple_of(i * tm, tm), tm)


def _kernel(x_hbm, wqkv_hbm, wo_hbm, win_hbm, wsp_hbm, bsp_ref, wout_hbm, c_ref, wmod_hbm,
            out_hbm,
            x_v, wqkv_v, wo_v, win_v, wsp_v, wout_v, wmod_v,
            wqvt_v, mod_v, k_v, qt_v, vt_v, ot_v, x1_v, z1_v, z2_v, bcol_v, obuf, h_v, zg_v, qb_v, kt_v, kb0, kb1,
            sems, osems, xsems, *, S, D, FH):
    DH = D // H
    NQ = S // TQ
    NKC = S // KC
    NU = H * NQ
    HPG = 128 // DH

    def cp(src, dst, n):
        return pltpu.make_async_copy(src, dst, sems.at[n])

    NB1 = S // TM1

    def cp_x(i):
        return pltpu.make_async_copy(x_hbm.at[_rows(i, TM1), :], x_v.at[_rows(i, TM1), :],
                                     xsems.at[i])

    cp_moda = cp(wmod_hbm.at[:, 0:2 * D], wmod_v.at[:, 0:2 * D], 0)
    cp_wk = cp(wqkv_hbm.at[:, D:2 * D], wqkv_v.at[:, D:2 * D], 2)
    cp_wq = cp(wqkv_hbm.at[:, 0:D], wqkv_v.at[:, 0:D], 3)
    cp_wv = cp(wqkv_hbm.at[:, 2 * D:3 * D], wqkv_v.at[:, 2 * D:3 * D], 4)
    cp_modb = cp(wmod_hbm.at[:, 2 * D:6 * D], wmod_v.at[:, 2 * D:6 * D], 6)
    cp_wo = cp(wo_hbm, wo_v, 7)
    cp_win = cp(win_hbm, win_v, 8)
    cp_wsp = cp(wsp_hbm, wsp_v, 9)
    cp_wout = cp(wout_hbm, wout_v, 10)
    late = (cp_modb, cp_wo, cp_win, cp_wsp, cp_wout)
    cp_x(0).start()
    for c_ in (cp_moda, cp_wq, cp_wv, cp_wk):
        c_.start()
    for i in range(1, NB1):
        cp_x(i).start()
    if not LATE_DMA:
        for c_ in late:
            c_.start()

    bcol_v[...] = jnp.transpose(jnp.broadcast_to(bsp_ref[...].astype(F32), (128, S)))
    cf = c_ref[...].astype(F32)
    sc = jnp.broadcast_to((cf * (1.0 / (1.0 + jnp.exp(-cf)))).astype(BF16), (8, D))

    cp_x(0).wait()
    xn0 = _layernorm(x_v[0:TM1, :].astype(F32))
    cp_moda.wait()
    mod_v[:, 0:2 * D] = jnp.dot(sc, wmod_v[:, 0:2 * D], preferred_element_type=F32)

    def modrow(i):
        return mod_v[0:1, i * D:(i + 1) * D]

    qscale = (DH ** -0.5) * math.log2(math.e)

    def affine1(xn):
        return (xn * (1.0 + modrow(1)) + modrow(0)).astype(BF16)

    h_v[0] = affine1(xn0)
    cp_wq.wait()
    wqvt_v[0:D, :] = jnp.transpose(wqkv_v[:, 0:D].astype(F32)).astype(BF16)
    cp_wv.wait()
    wqvt_v[D:2 * D, :] = jnp.transpose(wqkv_v[:, 2 * D:3 * D].astype(F32)).astype(BF16)
    cp_wk.wait()

    def p1_body(i, carry):
        nxt = jnp.minimum(i + 1, NB1 - 1)

        @pl.when(i + 1 < NB1)
        def _():
            cp_x(nxt).wait()

        h = h_v[i % 2]
        h_v[(i + 1) % 2] = affine1(_layernorm(x_v[_rows(nxt, TM1), :].astype(F32)))
        k32 = jnp.dot(h, wqkv_v[:, D:2 * D], preferred_element_type=F32)
        k = k32.astype(BF16)
        for g in range(D // 128):
            k_v[g, _rows(i, TM1), :] = k[:, g * 128:(g + 1) * 128]
        kt_v[i] = jnp.transpose(k32)
        for t in range(DH // NB1):
            d = i * (DH // NB1) + t
            row = kt_v[0, pl.ds(d, 1), :]
            kb0[0, d] = jnp.transpose(jnp.broadcast_to(row, (128, KV)))
        for c in range(TM1 // QVW):
            cols = pl.ds(pl.multiple_of(i * TM1 + c * QVW, QVW), QVW)
            qvt = lax.dot_general(wqvt_v[...], h[c * QVW:(c + 1) * QVW], (((1,), (1,)), ((), ())),
                                  preferred_element_type=F32)
            q32 = qvt[0:D] * qscale
            qt_v[:, cols] = q32.astype(BF16)
            vt_v[:, cols] = qvt[D:2 * D].astype(BF16)
            q3 = q32.reshape(D // 8, 8, QVW)
            for r in range(8):
                qr = jnp.broadcast_to(q3[:, r:r + 1, :], (D // 8, 8, QVW))
                for cc in range(QVW // 128):
                    qb_v[(i * TM1 + c * QVW) // 128 + cc, :, r] = qr[:, :, cc * 128:(cc + 1) * 128]
        return carry

    with jax.named_scope('p1'):
        lax.fori_loop(0, NB1, p1_body, 0)
    if LATE_DMA:
        for c_ in late:
            c_.start()

    def wq_masked(u):
        h = u // NQ
        qb = u % NQ
        q = qt_v[pl.ds(pl.multiple_of(h * DH, DH), DH), pl.ds(pl.multiple_of(qb * TQ, TQ), TQ)]
        qrep = jnp.concatenate([q] * HPG, axis=0)
        rows = lax.broadcasted_iota(jnp.int32, (128, TQ), 0)
        return jnp.where((rows // DH) == (h % HPG), qrep, jnp.zeros_like(qrep))

    def qk(u, kc, wq):
        g = (u // NQ) // HPG
        return jnp.dot(k_v[g, pl.ds(kc * KC, KC), :], wq, preferred_element_type=F32)

    def pv(u, kc, p):
        h = u // NQ
        vt = vt_v[pl.ds(pl.multiple_of(h * DH, DH), DH), pl.ds(kc * KC, KC)]
        return jnp.dot(vt, p.astype(BF16), preferred_element_type=F32)

    def red(x, op):
        return op(x.reshape(KC // 8, 8, TQ), axis=0)

    def store_o(u, acc, lsum):
        h = u // NQ
        qb = u % NQ
        ot_v[pl.ds(pl.multiple_of(h * DH, DH), DH),
             pl.ds(pl.multiple_of(qb * TQ, TQ), TQ)] = acc * (1.0 / lsum)

    NC = TQ // 128
    NSB = KV // SB
    sizes = [KC] * (S // KC)
    sizes[PVA] = KC // 2
    sizes[PVB] = KC // 2
    offs = [KV + sum(sizes[:c]) for c in range(len(sizes))]
    NSL = len(sizes)
    kbs = (kb0, kb1)

    def redn(x):
        return jnp.sum(x.reshape(x.shape[0] // 8, 8, TQ), axis=0)

    def fast_body(i, bad0):
      with jax.named_scope('p2it'):
        units = [(hh, qb) for hh in range(HPB) for qb in range(NQ)]
        NUU = len(units)
        n = NUU * NSL
        wqs, ss, acc, lsum, lv, pvp = {}, {}, {}, {}, {}, {}
        prev = [None]
        lagq, kdeps = [], []
        bad = [bad0]
        links = [(sb, c) for sb in range(NSB) for c in range(NC)]
        zctr = [0]

        def head(uu):
            return i * HPB + units[uu][0]

        def hrows(uu):
            return pl.ds(pl.multiple_of(head(uu) * DH, DH), DH)

        def qcols(uu):
            return pl.ds(units[uu][1] * TQ, TQ)

        def wq_static(uu):
            q = qt_v[hrows(uu), qcols(uu)]
            qrep = jnp.concatenate([q] * HPG, axis=0)
            rows = lax.broadcasted_iota(jnp.int32, (128, TQ), 0)
            return jnp.where((rows // DH) == (head(uu) % HPG), qrep, jnp.zeros_like(qrep))

        def pv2(uu, off, n_, p, dl=False):
            a = jnp.dot(vt_v[hrows(uu), pl.ds(off, n_)], p.astype(BF16),
                        preferred_element_type=F32)
            base = acc[uu] if uu in acc else bad[0] * 0.0
            if dl:
                kz = kdeps.pop()
                while kdeps:
                    kz = kz + kdeps.pop()
                kz = kz * 0.0
                base = base + jnp.concatenate(
                    [jnp.concatenate([kz] * NC, axis=1)] * (DH // 8), axis=0)
            acc[uu] = base + a

        def gen_kb(hn, kb, d):
            row = kt_v[0, pl.ds(hn * DH + d, 1), :]
            t = jnp.transpose(jnp.broadcast_to(row, (128, KV)))
            kb[0, d] = t
            return t[KV - 8:KV]

        def link(uu, sb, c, start, e):
            zctr[0] += 1
            z = lax.shift_right_logical(i + zctr[0], 16)
            hh, qb = units[uu]
            a = start
            for d in range(DH):
                kbd = kbs[hh % 2][z, d, sb * SB:(sb + 1) * SB, :].reshape(SB // 8, 8, 128)
                q = qb_v[qb * NC + c, head(uu) * (DH // 8) + d // 8 + z, d % 8]
                if e is not None and d == DH - 1:
                    q = q + e
                t = kbd * q[None]
                a = t if a is None else a + t
            return a

        def vpu_pv(uu, sb0, sb1):
            rows = [jnp.concatenate([pvp.pop((uu, sb, c)) for c in range(NC)], axis=1)
                    for sb in range(sb0, sb1)]
            pv2(uu, sb0 * SB, (sb1 - sb0) * SB, jnp.concatenate(rows, axis=0))

        def fin(uu):
            l = lsum.pop(uu) + jnp.concatenate([lv.pop((uu, c)) for c in range(NC)], axis=1)
            ls = jnp.sum(l, axis=0, keepdims=True)
            a = acc.pop(uu)
            ok = jnp.logical_and(jnp.logical_and(ls >= L_LO, ls <= L_HI), jnp.abs(a) <= F32_BIG)
            bad[0] = jnp.where(ok, bad[0], 1.0)
            ot_v[hrows(uu), qcols(uu)] = a * (1.0 / ls)

        for idx in range(n + 1):
            if idx < n:
                uu, kc = divmod(idx, NSL)
                if kc == 0:
                    wqs[uu] = wq_static(uu)
                ss[idx] = jnp.dot(k_v[head(uu) // HPG, pl.ds(offs[kc], sizes[kc]), :], wqs[uu],
                                  preferred_element_type=F32)
            if idx >= 1:
                uu, kc = divmod(idx - 1, NSL)
                hh, qb = units[uu]
                p = jnp.exp2(ss.pop(idx - 1))
                r = redn(p)
                lsum[uu] = r if kc == 0 else lsum[uu] + r
                pv2(uu, offs[kc], sizes[kc], p, dl=(idx - 1 == KBDL))
                hn = jnp.minimum(head(uu) + 1, H - 1)
                if hh == 0:
                    if kc < DH // NQ:
                        gen_kb(hn, kbs[1], qb * (DH // NQ) + kc)
                elif qb < DH // NSL:
                    kdeps.append(gen_kb(hn, kbs[0], qb * NSL + kc))
                lo = (kc * len(links)) // NSL
                hi = ((kc + 1) * len(links)) // NSL
                for li in range(lo, hi):
                    sb, c = links[li]
                    e = lagq.pop(0) if len(lagq) >= LAG else None
                    a = link(uu, sb, c, prev[0], e)
                    pe = jnp.exp2(a)
                    ls = jnp.sum(pe, axis=0)
                    key = (uu, c)
                    lv[key] = ls if key not in lv else lv[key] + ls
                    pvp[(uu, sb, c)] = pe.reshape(SB, 128)
                    prev[0] = a[0:1] * 0.0
                    lagq.append(jnp.minimum(lv[key], 0.0))
                if uu >= 1:
                    if kc == PVA:
                        vpu_pv(uu - 1, 0, NSB // 2)
                    if kc == PVB:
                        vpu_pv(uu - 1, NSB // 2, NSB)
                        fin(uu - 1)
        vpu_pv(NUU - 1, 0, NSB)
        fin(NUU - 1)
        return bad[0]

    with jax.named_scope('p2'):
        bad = lax.fori_loop(0, H // HPB, fast_body, jnp.zeros((DH, TQ), F32))
    any_bad = jnp.max(bad) > (-1.0 if FORCE_SAFE else 0.0)

    @pl.when(any_bad)
    def _():
        def safe_body(u, carry):
            wq = wq_masked(u)
            acc = l = m = None
            for kc in range(NKC):
                s = qk(u, kc, wq)
                mc = jnp.max(red(s, jnp.max), axis=0, keepdims=True)
                if kc == 0:
                    m = mc
                    p = jnp.exp2(s - m)
                    acc = pv(u, kc, p)
                    l = red(p, jnp.sum)
                else:
                    mn = jnp.maximum(m, mc)
                    al = jnp.exp2(m - mn)
                    p = jnp.exp2(s - mn)
                    acc = acc * al + pv(u, kc, p)
                    l = l * al + red(p, jnp.sum)
                    m = mn
            store_o(u, acc, jnp.sum(l, axis=0, keepdims=True))
            return carry

        lax.fori_loop(0, NU, safe_body, 0)

    cp_modb.wait()
    cp_wo.wait()
    cp_win.wait()
    mod_v[:, 2 * D:6 * D] = jnp.dot(sc, wmod_v[:, 2 * D:6 * D], preferred_element_type=F32)

    NB3 = S // TM3

    def p3_a(i):
        rows = _rows(i, TM3)
        o = jnp.transpose(ot_v[:, rows]).astype(BF16)
        a = jnp.dot(o, wo_v[...], preferred_element_type=F32)
        x1 = x_v[rows, :].astype(F32) + modrow(2) * a
        x1_v[rows, :] = x1
        return (_layernorm(x1) * (1.0 + modrow(4)) + modrow(3)).astype(BF16)

    def p3_body(j, h2):
        for t in range(U3):
            i = j * U3 + t
            rows = _rows(i, TM3)
            nxt = p3_a(jnp.minimum(i + 1, NB3 - 1))
            zg_v[t % 2] = _gelu(jnp.dot(h2, win_v[:, FH:2 * FH], preferred_element_type=F32))
            if FAKE3:
                keep = lax.broadcasted_iota(jnp.int32, (TM3, D), 1) >= lax.shift_right_logical(j, 16)
                h2b = jnp.where(keep, h2, nxt)
            else:
                h2b = h2
            z1_v[rows, :] = _gelu(jnp.dot(h2b, win_v[:, 0:FH], preferred_element_type=F32))
            z = lax.shift_right_logical(j, 16 + t)
            zg = zg_v[t % 2, pl.ds(pl.multiple_of(z * 8, 8), TM3), :]
            z2_v[rows, :] = _layernorm(zg).astype(BF16)
            h2 = nxt
        return h2

    with jax.named_scope('p3'):
        lax.fori_loop(0, NB3 // U3, p3_body, p3_a(0))

    cp_wsp.wait()
    cp_wout.wait()
    NB4 = S // TM4

    def out_copy(i):
        return pltpu.make_async_copy(obuf.at[_rows(i, TM4), :], out_hbm.at[_rows(i, TM4), :],
                                     osems.at[i])

    def p4_g(i):
        rows = _rows(i, TM4)
        g = jnp.dot(wsp_v[rows, :], z2_v[...], preferred_element_type=F32)
        b = bcol_v[rows, :]
        g = g + jnp.concatenate([b] * (FH // 128), axis=1)
        return (z1_v[rows, :] * g).astype(BF16)

    def p4_y(i, t):
        rows = _rows(i, TM4)
        y = jnp.dot(t, wout_v[...], preferred_element_type=F32)
        obuf[rows, :] = (x1_v[rows, :] + modrow(5) * y).astype(BF16)

    def p4_group(idxs):
        for i in idxs:
            p4_y(i, p4_g(i))
        for i in idxs:
            out_copy(i).start()

    with jax.named_scope('p4'):
        _loop(NB4, U4, p4_group)
    for i in range(NB4):
        out_copy(i).wait()


@jax.jit
def pallas_adaLN_cond__softmax_full_mha__mixer_gmlp__prompt_kernel(
    A_x, A_wqkv, A_wo, B_x, B_w_in, B_w_sp, B_b_sp, B_w_out, c, w_mod,
):
    B, S, D = A_x.shape
    F = B_w_in.shape[-1]
    FH = F // 2
    any_spec = pl.BlockSpec(memory_space=pl.ANY)
    vmem_spec = pl.BlockSpec(memory_space=pltpu.VMEM)
    out = pl.pallas_call(
        functools.partial(_kernel, S=S, D=D, FH=FH),
        out_shape=jax.ShapeDtypeStruct((S, D), BF16),
        in_specs=[any_spec, any_spec, any_spec, any_spec, any_spec, vmem_spec,
                  any_spec, vmem_spec, any_spec],
        out_specs=any_spec,
        scratch_shapes=[
            pltpu.VMEM((S, D), BF16),
            pltpu.VMEM((D, 3 * D), BF16),
            pltpu.VMEM((D, D), BF16),
            pltpu.VMEM((D, F), BF16),
            pltpu.VMEM((S, S), BF16),
            pltpu.VMEM((FH, D), BF16),
            pltpu.VMEM((D, 6 * D), BF16),
            pltpu.VMEM((2 * D, D), BF16),
            pltpu.VMEM((8, 6 * D), F32),
            pltpu.VMEM((D // 128, S, 128), BF16),
            pltpu.VMEM((D, S), BF16),
            pltpu.VMEM((D, S), BF16),
            pltpu.VMEM((D, S), F32),
            pltpu.VMEM((S, D), F32),
            pltpu.VMEM((S, FH), F32),
            pltpu.VMEM((S, FH), BF16),
            pltpu.VMEM((S, 128), F32),
            pltpu.VMEM((S, D), BF16),
            pltpu.VMEM((2, TM1, D), BF16),
            pltpu.VMEM((2, TM3, FH), F32),
            pltpu.VMEM((S // 128, D // 8, 8, 8, 128), F32),
            pltpu.VMEM((S // TM1, D, TM1), F32),
            pltpu.VMEM((1, D // H, KV, 128), F32),
            pltpu.VMEM((1, D // H, KV, 128), F32),
            pltpu.SemaphoreType.DMA((11,)),
            pltpu.SemaphoreType.DMA((S // TM4,)),
            pltpu.SemaphoreType.DMA((S // TM1,)),
        ],
        compiler_params=pltpu.CompilerParams(vmem_limit_bytes=112 * 1024 * 1024),
    )(A_x.reshape(S, D), A_wqkv, A_wo, B_w_in, B_w_sp, B_b_sp.reshape(1, S), B_w_out, c, w_mod)
    return out.reshape(B, S, D)
```

```python
import functools
import math

import jax
import jax.numpy as jnp
from jax import lax
import jax.experimental.pallas as pl
import jax.experimental.pallas.tpu as pltpu

F32 = jnp.float32
BF16 = jnp.bfloat16

H = 32
EPS = 1e-5
TM = 256
TQ = 512
KC = 256
KV = 256
SB = 32
HPB = 2
LAG = 2
PVA, PVB = 0, 2
KBDL = 56
LNP = 128

L_LO = 2.0 ** -32
L_HI = 2.0 ** 64
F32_BIG = 3.0e38


def _layernorm(x):
    m = jnp.mean(x, axis=-1, keepdims=True)
    xc = x - m
    v = jnp.mean(xc * xc, axis=-1, keepdims=True)
    return xc * lax.rsqrt(v + EPS)


def _layernorm_pieces(load, nrows, piece, width, emit):
    dep = None
    for r0 in range(0, nrows, piece):
        x = load(r0, piece)
        s = x[:, 0:128] if dep is None else x[:, 0:128] + dep
        for c in range(1, width // 128):
            s = s + x[:, c * 128:(c + 1) * 128]
        m = jnp.sum(s, axis=-1, keepdims=True) * (1.0 / width)
        xc = x - m
        sq = xc * xc
        v = sq[:, 0:128]
        for c in range(1, width // 128):
            v = v + sq[:, c * 128:(c + 1) * 128]
        v = jnp.sum(v, axis=-1, keepdims=True) * (1.0 / width)
        y = xc * lax.rsqrt(v + EPS)
        emit(r0, y)
        dep = y[:, width - 128:width] * 0.0


def _gelu(x):
    c = math.sqrt(2.0 / math.pi)
    return 0.5 * x * (1.0 + jnp.tanh(x * (c + (c * 0.044715) * (x * x))))


def _rows(i, n, off=0):
    if isinstance(i, int):
        return pl.ds(i * TM + off, n)
    return pl.ds(pl.multiple_of(i * TM + off, math.gcd(TM, off)), n)


def _kernel(x_hbm, wqkv_hbm, wo_hbm, win_hbm, wsp_hbm, bsp_hbm, wout_hbm, c_hbm, wmod_hbm,
            out_hbm,
            x_v, wqkv_v, wo_v, win_v, wsp_v, wout_v, wmod_v,
            wqvt_v, mod_v, k_v, qt_v, vt_v, ot_v, x1_v, z1_v, z2_v, bcol_v, obuf,
            h1_v, ha_v, hb_v, zga_v, zgb_v, qb_v, kt_v, kb0, kb1, bsp_v, c_v, sc_v,
            sems, xsems, osems, *, S, D, FH):
    DH = D // H
    NQ = S // TQ
    NB = S // TM
    HPG = 128 // DH
    NC = TQ // 128

    def cp(src, dst, n):
        return pltpu.make_async_copy(src, dst, sems.at[n])

    def cp_x(i):
        return pltpu.make_async_copy(x_hbm.at[_rows(i, TM), :], x_v.at[_rows(i, TM), :],
                                     xsems.at[i])

    cp_c = cp(c_hbm, c_v, 0)
    cp_b = cp(bsp_hbm, bsp_v, 1)
    cp_moda = cp(wmod_hbm.at[:, 0:2 * D], wmod_v.at[:, 0:2 * D], 2)
    cp_wq = cp(wqkv_hbm.at[:, 0:D], wqkv_v.at[:, 0:D], 3)
    cp_wv = cp(wqkv_hbm.at[:, 2 * D:3 * D], wqkv_v.at[:, 2 * D:3 * D], 4)
    cp_wk = cp(wqkv_hbm.at[:, D:2 * D], wqkv_v.at[:, D:2 * D], 5)
    cp_modb = cp(wmod_hbm.at[:, 2 * D:6 * D], wmod_v.at[:, 2 * D:6 * D], 6)
    cp_wo = cp(wo_hbm, wo_v, 7)
    cp_win = cp(win_hbm, win_v, 8)
    cp_wsp = cp(wsp_hbm, wsp_v, 9)
    cp_wout = cp(wout_hbm, wout_v, 10)

    cp_b.start()
    cp_c.start()
    cp_x(0).start()
    cp_moda.start()
    cp_b.wait()
    bcol_v[...] = jnp.transpose(
        jnp.broadcast_to(bsp_v[...].astype(F32).reshape(1, S), (128, S)))
    cp_c.wait()
    cf = c_v[...].astype(F32)
    sc_v[...] = jnp.broadcast_to(cf * (1.0 / (1.0 + jnp.exp(-cf))), (8, D))
    cp_x(0).wait()
    cp_wq.start()
    xn0 = _layernorm(x_v[0:TM, :].astype(F32))
    cp_moda.wait()
    cp_wv.start()
    mod_v[:, 0:2 * D] = jnp.dot(sc_v[...].astype(BF16), wmod_v[:, 0:2 * D],
                                preferred_element_type=F32)

    def modrow(i):
        return mod_v[0:1, i * D:(i + 1) * D]

    def affine1(xn):
        return (xn * (1.0 + modrow(1)) + modrow(0)).astype(BF16)

    h1_v[0] = affine1(xn0)
    cp_wq.wait()
    cp_wk.start()
    cp_x(1).start()
    wqvt_v[0:D, :] = jnp.transpose(wqkv_v[:, 0:D].astype(F32)).astype(BF16)
    cp_wv.wait()
    cp_x(2).start()
    wqvt_v[D:2 * D, :] = jnp.transpose(wqkv_v[:, 2 * D:3 * D].astype(F32)).astype(BF16)
    cp_wk.wait()
    for i in range(3, NB):
        cp_x(i).start()
    cp_modb.start()

    qscale = (DH ** -0.5) * math.log2(math.e)

    def bcast_key_column(row):
        return jnp.transpose(jnp.broadcast_to(row, (128, KV)))

    def p1_body(i, carry):
        nxt = jnp.minimum(i + 1, NB - 1)

        @pl.when(i + 1 < NB)
        def _():
            cp_x(nxt).wait()

        h = h1_v[i % 2]
        h1_v[(i + 1) % 2] = affine1(_layernorm(x_v[_rows(nxt, TM), :].astype(F32)))
        k32 = jnp.dot(h, wqkv_v[:, D:2 * D], preferred_element_type=F32)
        k = k32.astype(BF16)
        for g in range(D // 128):
            k_v[g, _rows(i, TM), :] = k[:, g * 128:(g + 1) * 128]
        kt_v[i] = jnp.transpose(k32)
        for t in range(DH // NB):
            d = i * (DH // NB) + t
            kb0[0, d] = bcast_key_column(kt_v[0, pl.ds(d, 1), :])
        for c in range(TM // 128):
            cols = _rows(i, 128, c * 128)
            qvt = lax.dot_general(wqvt_v[...], h[c * 128:(c + 1) * 128],
                                  (((1,), (1,)), ((), ())), preferred_element_type=F32)
            q32 = qvt[0:D] * qscale
            qt_v[:, cols] = q32.astype(BF16)
            vt_v[:, cols] = qvt[D:2 * D].astype(BF16)
            q3 = q32.reshape(D // 8, 8, 128)
            for r in range(8):
                qb_v[i * (TM // 128) + c, :, r] = jnp.broadcast_to(q3[:, r:r + 1, :],
                                                                   (D // 8, 8, 128))
        return carry

    lax.fori_loop(0, NB, p1_body, 0)
    for c_ in (cp_wo, cp_win, cp_wsp, cp_wout):
        c_.start()

    NSB = KV // SB
    sizes = [KC] * (S // KC)
    sizes[PVA] = KC // 2
    sizes[PVB] = KC // 2
    offs = [KV + sum(sizes[:c]) for c in range(len(sizes))]
    NSL = len(sizes)
    kbs = (kb0, kb1)

    def hrows(h):
        return pl.ds(pl.multiple_of(h * DH, DH), DH)

    def masked_q(h, cols):
        q = qt_v[hrows(h), cols]
        qrep = jnp.concatenate([q] * HPG, axis=0)
        rows = lax.broadcasted_iota(jnp.int32, (128, TQ), 0)
        return jnp.where((rows // DH) == (h % HPG), qrep, jnp.zeros_like(qrep))

    def fold(x, op):
        return op(x.reshape(x.shape[0] // 8, 8, TQ), axis=0)

    def fast_body(i, bad0):
        units = [(hh, qb) for hh in range(HPB) for qb in range(NQ)]
        NUU = len(units)
        n = NUU * NSL
        wqs, ss, acc, lsum, lv, pvp = {}, {}, {}, {}, {}, {}
        prev = [None]
        lagq, kdeps = [], []
        bad = [bad0]
        links = [(sb, c) for sb in range(NSB) for c in range(NC)]
        zctr = [0]

        def head(uu):
            return i * HPB + units[uu][0]

        def qcols(uu):
            return pl.ds(units[uu][1] * TQ, TQ)

        def pv(uu, off, n_, p, deadline=False):
            a = jnp.dot(vt_v[hrows(head(uu)), pl.ds(off, n_)], p.astype(BF16),
                        preferred_element_type=F32)
            base = acc[uu] if uu in acc else bad[0] * 0.0
            if deadline:
                kz = kdeps.pop()
                while kdeps:
                    kz = kz + kdeps.pop()
                kz = kz * 0.0
                base = base + jnp.concatenate(
                    [jnp.concatenate([kz] * NC, axis=1)] * (DH // 8), axis=0)
            acc[uu] = base + a

        def gen_kb(hn, kb, d):
            t = bcast_key_column(kt_v[0, pl.ds(hn * DH + d, 1), :])
            kb[0, d] = t
            return t[KV - 8:KV]

        def link(uu, sb, c, start, e):
            zctr[0] += 1
            z = lax.shift_right_logical(i + zctr[0], 16)
            hh, qb = units[uu]
            a = start
            for d in range(DH):
                kbd = kbs[hh % 2][z, d, sb * SB:(sb + 1) * SB, :].reshape(SB // 8, 8, 128)
                q = qb_v[qb * NC + c, head(uu) * (DH // 8) + d // 8 + z, d % 8]
                if e is not None and d == DH - 1:
                    q = q + e
                t = kbd * q[None]
                a = t if a is None else a + t
            return a

        def vpu_pv(uu, sb0, sb1):
            rows = [jnp.concatenate([pvp.pop((uu, sb, c)) for c in range(NC)], axis=1)
                    for sb in range(sb0, sb1)]
            pv(uu, sb0 * SB, (sb1 - sb0) * SB, jnp.concatenate(rows, axis=0))

        def fin(uu):
            l = lsum.pop(uu) + jnp.concatenate([lv.pop((uu, c)) for c in range(NC)], axis=1)
            ls = jnp.sum(l, axis=0, keepdims=True)
            a = acc.pop(uu)
            ok = jnp.logical_and(jnp.logical_and(ls >= L_LO, ls <= L_HI), jnp.abs(a) <= F32_BIG)
            bad[0] = jnp.where(ok, bad[0], 1.0)
            ot_v[hrows(head(uu)), qcols(uu)] = a * (1.0 / ls)

        for idx in range(n + 1):
            if idx < n:
                uu, kc = divmod(idx, NSL)
                if kc == 0:
                    wqs[uu] = masked_q(head(uu), qcols(uu))
                ss[idx] = jnp.dot(k_v[head(uu) // HPG, pl.ds(offs[kc], sizes[kc]), :], wqs[uu],
                                  preferred_element_type=F32)
            if idx >= 1:
                uu, kc = divmod(idx - 1, NSL)
                hh, qb = units[uu]
                p = jnp.exp2(ss.pop(idx - 1))
                r = fold(p, jnp.sum)
                lsum[uu] = r if kc == 0 else lsum[uu] + r
                pv(uu, offs[kc], sizes[kc], p, deadline=(idx - 1 == KBDL))
                hn = jnp.minimum(head(uu) + 1, H - 1)
                if hh == 0:
                    if kc < DH // NQ:
                        gen_kb(hn, kbs[1], qb * (DH // NQ) + kc)
                elif qb < DH // NSL:
                    kdeps.append(gen_kb(hn, kbs[0], qb * NSL + kc))
                lo = (kc * len(links)) // NSL
                hi = ((kc + 1) * len(links)) // NSL
                for li in range(lo, hi):
                    sb, c = links[li]
                    e = lagq.pop(0) if len(lagq) >= LAG else None
                    a = link(uu, sb, c, prev[0], e)
                    pe = jnp.exp2(a)
                    ls = jnp.sum(pe, axis=0)
                    key = (uu, c)
                    lv[key] = ls if key not in lv else lv[key] + ls
                    pvp[(uu, sb, c)] = pe.reshape(SB, 128)
                    prev[0] = a[0:1] * 0.0
                    lagq.append(jnp.minimum(lv[key], 0.0))
                if uu >= 1:
                    if kc == PVA:
                        vpu_pv(uu - 1, 0, NSB // 2)
                    if kc == PVB:
                        vpu_pv(uu - 1, NSB // 2, NSB)
                        fin(uu - 1)
        vpu_pv(NUU - 1, 0, NSB)
        fin(NUU - 1)
        return bad[0]

    bad = lax.fori_loop(0, H // HPB, fast_body, jnp.zeros((DH, TQ), F32))
    cp_modb.wait()
    mod_v[:, 2 * D:6 * D] = jnp.dot(sc_v[...].astype(BF16), wmod_v[:, 2 * D:6 * D],
                                    preferred_element_type=F32)

    @pl.when(jnp.max(bad) > 0.0)
    def _():
        def safe_body(u, carry):
            h = u // NQ
            cols = pl.ds(pl.multiple_of((u % NQ) * TQ, TQ), TQ)
            wq = masked_q(h, cols)
            acc = l = m = None
            for kc in range(S // KC):
                keys = pl.ds(kc * KC, KC)
                s = jnp.dot(k_v[h // HPG, keys, :], wq, preferred_element_type=F32)
                mc = jnp.max(fold(s, jnp.max), axis=0, keepdims=True)
                mn = mc if kc == 0 else jnp.maximum(m, mc)
                p = jnp.exp2(s - mn)
                a = jnp.dot(vt_v[hrows(h), keys], p.astype(BF16), preferred_element_type=F32)
                r = fold(p, jnp.sum)
                if kc == 0:
                    acc, l = a, r
                else:
                    al = jnp.exp2(m - mn)
                    acc, l = acc * al + a, l * al + r
                m = mn
            ot_v[hrows(h), cols] = acc * (1.0 / jnp.sum(l, axis=0, keepdims=True))
            return carry

        lax.fori_loop(0, H * NQ, safe_body, 0)

    cp_wo.wait()
    cp_win.wait()
    hbufs = (ha_v, hb_v)
    zbufs = (zga_v, zgb_v)

    def p3_a(i, hbuf):
        rows = _rows(i, TM)
        o = jnp.transpose(ot_v[:, rows]).astype(BF16)
        a = jnp.dot(o, wo_v[...], preferred_element_type=F32)
        x1 = x_v[rows, :].astype(F32) + modrow(2) * a
        x1_v[rows, :] = x1

        def emit(r0, y):
            hbuf[r0:r0 + LNP, :] = (y * (1.0 + modrow(4)) + modrow(3)).astype(BF16)

        _layernorm_pieces(lambda r0, n: x1[r0:r0 + n], TM, LNP, D, emit)

    def p3_block(i, t, z, with_next=True):
        h2 = hbufs[t][...]
        zbufs[t][0] = _gelu(jnp.dot(h2, win_v[:, FH:2 * FH], preferred_element_type=F32))
        if with_next:
            p3_a(i + 1, hbufs[1 - t])
        z1_v[_rows(i, TM), :] = jnp.dot(h2, win_v[:, 0:FH], preferred_element_type=F32)

        def emit(r0, y):
            z2_v[_rows(i, LNP, r0), :] = y.astype(BF16)

        _layernorm_pieces(lambda r0, n: zbufs[t][z, r0:r0 + n, :], TM, LNP, FH, emit)

    def p3_body(j, carry):
        for t in range(2):
            p3_block(j * 2 + t, t, lax.shift_right_logical(j, 16 + t))
        return carry

    p3_a(0, hbufs[0])
    zo = lax.fori_loop(0, NB // 2 - 1, p3_body, jnp.int32(0))
    p3_block(NB - 2, 0, zo)
    p3_block(NB - 1, 1, zo, with_next=False)

    cp_wsp.wait()
    cp_wout.wait()

    def out_copy(i):
        return pltpu.make_async_copy(obuf.at[_rows(i, TM), :], out_hbm.at[_rows(i, TM), :],
                                     osems.at[i])

    def p4_body(i, carry):
        rows = _rows(i, TM)
        g = jnp.dot(wsp_v[rows, :], z2_v[...], preferred_element_type=F32)
        g = g + jnp.concatenate([bcol_v[rows, :]] * (FH // 128), axis=1)
        t = (_gelu(z1_v[rows, :]) * g).astype(BF16)
        y = jnp.dot(t, wout_v[...], preferred_element_type=F32)
        obuf[rows, :] = (x1_v[rows, :] + modrow(5) * y).astype(BF16)
        out_copy(i).start()
        return carry

    lax.fori_loop(0, NB, p4_body, 0)
    for i in range(NB):
        out_copy(i).wait()


@jax.jit
def pallas_adaLN_cond__softmax_full_mha__mixer_gmlp__prompt_kernel(
    A_x: jax.Array,
    A_wqkv: jax.Array,
    A_wo: jax.Array,
    B_x: jax.Array,
    B_w_in: jax.Array,
    B_w_sp: jax.Array,
    B_b_sp: jax.Array,
    B_w_out: jax.Array,
    c: jax.Array,
    w_mod: jax.Array,
):
    B, S, D = A_x.shape
    F = B_w_in.shape[-1]
    FH = F // 2
    DH = D // H
    assert B == 1 and KV == TM
    any_spec = pl.BlockSpec(memory_space=pl.ANY)
    out = pl.pallas_call(
        functools.partial(_kernel, S=S, D=D, FH=FH),
        out_shape=jax.ShapeDtypeStruct((S, D), BF16),
        in_specs=[any_spec] * 9,
        out_specs=any_spec,
        scratch_shapes=[
            pltpu.VMEM((S, D), BF16),
            pltpu.VMEM((D, 3 * D), BF16),
            pltpu.VMEM((D, D), BF16),
            pltpu.VMEM((D, F), BF16),
            pltpu.VMEM((S, S), BF16),
            pltpu.VMEM((FH, D), BF16),
            pltpu.VMEM((D, 6 * D), BF16),
            pltpu.VMEM((2 * D, D), BF16),
            pltpu.VMEM((8, 6 * D), F32),
            pltpu.VMEM((D // 128, S, 128), BF16),
            pltpu.VMEM((D, S), BF16),
            pltpu.VMEM((D, S), BF16),
            pltpu.VMEM((D, S), F32),
            pltpu.VMEM((S, D), F32),
            pltpu.VMEM((S, FH), F32),
            pltpu.VMEM((S, FH), BF16),
            pltpu.VMEM((S, 128), F32),
            pltpu.VMEM((S, D), BF16),
            pltpu.VMEM((2, TM, D), BF16),
            pltpu.VMEM((TM, D), BF16),
            pltpu.VMEM((TM, D), BF16),
            pltpu.VMEM((1, TM, FH), F32),
            pltpu.VMEM((1, TM, FH), F32),
            pltpu.VMEM((S // 128, D // 8, 8, 8, 128), F32),
            pltpu.VMEM((S // TM, D, TM), F32),
            pltpu.VMEM((1, DH, KV, 128), F32),
            pltpu.VMEM((1, DH, KV, 128), F32),
            pltpu.VMEM((S,), BF16),
            pltpu.VMEM((1, D), BF16),
            pltpu.VMEM((8, D), F32),
            pltpu.SemaphoreType.DMA((11,)),
            pltpu.SemaphoreType.DMA((S // TM,)),
            pltpu.SemaphoreType.DMA((S // TM,)),
        ],
        compiler_params=pltpu.CompilerParams(vmem_limit_bytes=112 * 1024 * 1024),
    )(A_x.reshape(S, D), A_wqkv, A_wo, B_w_in, B_w_sp, B_b_sp, B_w_out, c, w_mod)
    return out.reshape(B, S, D)
```

```python
import functools
import math

import jax
import jax.numpy as jnp
from jax import lax
import jax.experimental.pallas as pl
import jax.experimental.pallas.tpu as pltpu

F32 = jnp.float32
BF16 = jnp.bfloat16

H = 32
EPS = 1e-5
TM = 256
TQ = 512
KC = 256
KV = 256
SB = 32
HPB = 2
LAG = 2
PVA, PVB = 1, 3
KBDL = 48
LNP = 128

L_LO = 2.0 ** -32
L_HI = 2.0 ** 64
F32_BIG = 3.0e38


def _layernorm(x):
    m = jnp.mean(x, axis=-1, keepdims=True)
    xc = x - m
    v = jnp.mean(xc * xc, axis=-1, keepdims=True)
    return xc * lax.rsqrt(v + EPS)


def _layernorm_pieces(load, nrows, piece, width, emit):
    dep = None
    for r0 in range(0, nrows, piece):
        x = load(r0, piece)
        s = x[:, 0:128] if dep is None else x[:, 0:128] + dep
        for c in range(1, width // 128):
            s = s + x[:, c * 128:(c + 1) * 128]
        m = jnp.sum(s, axis=-1, keepdims=True) * (1.0 / width)
        xc = x - m
        sq = xc * xc
        v = sq[:, 0:128]
        for c in range(1, width // 128):
            v = v + sq[:, c * 128:(c + 1) * 128]
        v = jnp.sum(v, axis=-1, keepdims=True) * (1.0 / width)
        y = xc * lax.rsqrt(v + EPS)
        emit(r0, y)
        dep = y[:, width - 128:width] * 0.0


def _gelu(x):
    c = math.sqrt(2.0 / math.pi)
    return 0.5 * x * (1.0 + jnp.tanh(x * (c + (c * 0.044715) * (x * x))))


def _rows(i, n, off=0):
    if isinstance(i, int):
        return pl.ds(i * TM + off, n)
    return pl.ds(pl.multiple_of(i * TM + off, math.gcd(TM, off)), n)


def _kernel(x_hbm, wqkv_hbm, wo_hbm, win_hbm, wsp_hbm, bsp_hbm, wout_hbm, c_hbm, wmod_hbm,
            out_hbm,
            x_v, wqkv_v, wo_v, win_v, wsp_v, wout_v, wmod_v,
            wqvt_v, mod_v, k_v, qt_v, vt_v, ot_v, x1_v, z1_v, z2_v, bcol_v, obuf,
            h1_v, ha_v, hb_v, zga_v, zgb_v, qb_v, kt_v, kb0, kb1, bsp_v, c_v, sc_v,
            sems, xsems, osems, *, S, D, FH):
    DH = D // H
    NQ = S // TQ
    NB = S // TM
    HPG = 128 // DH
    NC = TQ // 128

    def cp(src, dst, n):
        return pltpu.make_async_copy(src, dst, sems.at[n])

    def cp_x(i):
        return pltpu.make_async_copy(x_hbm.at[_rows(i, TM), :], x_v.at[_rows(i, TM), :],
                                     xsems.at[i])

    cp_c = cp(c_hbm, c_v, 0)
    cp_b = cp(bsp_hbm, bsp_v, 1)
    cp_moda = cp(wmod_hbm.at[:, 0:2 * D], wmod_v.at[:, 0:2 * D], 2)
    cp_wq = cp(wqkv_hbm.at[:, 0:D], wqkv_v.at[:, 0:D], 3)
    cp_wv = cp(wqkv_hbm.at[:, 2 * D:3 * D], wqkv_v.at[:, 2 * D:3 * D], 4)
    cp_wk = cp(wqkv_hbm.at[:, D:2 * D], wqkv_v.at[:, D:2 * D], 5)
    cp_modb = cp(wmod_hbm.at[:, 2 * D:6 * D], wmod_v.at[:, 2 * D:6 * D], 6)
    cp_wo = cp(wo_hbm, wo_v, 7)
    cp_win = cp(win_hbm, win_v, 8)
    cp_wsp = cp(wsp_hbm, wsp_v, 9)
    cp_wout = cp(wout_hbm, wout_v, 10)

    cp_b.start()
    cp_c.start()
    cp_x(0).start()
    cp_moda.start()
    cp_b.wait()
    bcol_v[...] = jnp.transpose(
        jnp.broadcast_to(bsp_v[...].astype(F32).reshape(1, S), (128, S)))
    cp_c.wait()
    cf = c_v[...].astype(F32)
    sc_v[...] = jnp.broadcast_to(cf * (1.0 / (1.0 + jnp.exp(-cf))), (8, D))
    cp_x(0).wait()
    cp_wq.start()
    xn0 = _layernorm(x_v[0:TM, :].astype(F32))
    cp_moda.wait()
    cp_wv.start()
    mod_v[:, 0:2 * D] = jnp.dot(sc_v[...].astype(BF16), wmod_v[:, 0:2 * D],
                                preferred_element_type=F32)

    def modrow(i):
        return mod_v[0:1, i * D:(i + 1) * D]

    def affine1(xn):
        return (xn * (1.0 + modrow(1)) + modrow(0)).astype(BF16)

    h1_v[0] = affine1(xn0)
    cp_wq.wait()
    cp_wk.start()
    cp_x(1).start()
    wqvt_v[:, 0] = jnp.transpose(wqkv_v[:, 0:D].astype(F32)).astype(BF16).reshape(H, DH, D)
    cp_wv.wait()
    cp_x(2).start()
    wqvt_v[:, 1] = jnp.transpose(
        wqkv_v[:, 2 * D:3 * D].astype(F32)).astype(BF16).reshape(H, DH, D)
    cp_wk.wait()
    for i in range(3, NB):
        cp_x(i).start()
    cp_modb.start()

    qscale = (DH ** -0.5) * math.log2(math.e)

    def bcast_key_column(row):
        return jnp.transpose(jnp.broadcast_to(row, (128, KV)))

    def p1_body(i, carry):
        nxt = jnp.minimum(i + 1, NB - 1)

        @pl.when(i + 1 < NB)
        def _():
            cp_x(nxt).wait()

        h = h1_v[i % 2]
        h1_v[(i + 1) % 2] = affine1(_layernorm(x_v[_rows(nxt, TM), :].astype(F32)))
        k32 = jnp.dot(h, wqkv_v[:, D:2 * D], preferred_element_type=F32)
        k = k32.astype(BF16)
        for g in range(D // 128):
            k_v[g, _rows(i, TM), :] = k[:, g * 128:(g + 1) * 128]
        kt_v[i] = jnp.transpose(k32)
        for t in range(DH // NB):
            d = i * (DH // NB) + t
            kb0[0, d] = bcast_key_column(kt_v[0, pl.ds(d, 1), :])
        for c in range(TM // 128):
            cols = _rows(i, 128, c * 128)
            qvt = lax.dot_general(wqvt_v[...].reshape(2 * D, D), h[c * 128:(c + 1) * 128],
                                  (((1,), (1,)), ((), ())), preferred_element_type=F32)
            qvt = qvt.reshape(H, 2, DH, 128)
            q32 = qvt[:, 0].reshape(D, 128) * qscale
            qt_v[:, cols] = q32.astype(BF16)
            vt_v[:, cols] = qvt[:, 1].reshape(D, 128).astype(BF16)
            q3 = q32.reshape(D // 8, 8, 128)
            for r in range(8):
                qb_v[i * (TM // 128) + c, :, r] = jnp.broadcast_to(q3[:, r:r + 1, :],
                                                                   (D // 8, 8, 128))
        return carry

    lax.fori_loop(0, NB, p1_body, 0)
    for c_ in (cp_wo, cp_win, cp_wsp, cp_wout):
        c_.start()

    NSB = KV // SB
    sizes = [KC] * (S // KC)
    sizes[PVA] = KC // 2
    sizes[PVB] = KC // 2
    offs = [KV + sum(sizes[:c]) for c in range(len(sizes))]
    NSL = len(sizes)
    kbs = (kb0, kb1)

    def hrows(h):
        return pl.ds(pl.multiple_of(h * DH, DH), DH)

    def masked_q(h, cols):
        q = qt_v[hrows(h), cols]
        qrep = jnp.concatenate([q] * HPG, axis=0)
        rows = lax.broadcasted_iota(jnp.int32, (128, TQ), 0)
        return jnp.where((rows // DH) == (h % HPG), qrep, jnp.zeros_like(qrep))

    def fold(x, op):
        return op(x.reshape(x.shape[0] // 8, 8, TQ), axis=0)

    def fast_body(i, bad0):
        units = [(hh, qb) for hh in range(HPB) for qb in range(NQ)]
        NUU = len(units)
        n = NUU * NSL
        wqs, ss, acc, lsum, lv, pvp = {}, {}, {}, {}, {}, {}
        prev = [None]
        lagq, kdeps = [], []
        bad = [bad0]
        links = [(sb, c) for sb in range(NSB) for c in range(NC)]
        zctr = [0]

        def head(uu):
            return i * HPB + units[uu][0]

        def qcols(uu):
            return pl.ds(units[uu][1] * TQ, TQ)

        def pv(uu, off, n_, p, deadline=False):
            a = jnp.dot(vt_v[hrows(head(uu)), pl.ds(off, n_)], p.astype(BF16),
                        preferred_element_type=F32)
            base = acc[uu] if uu in acc else bad[0] * 0.0
            if deadline:
                kz = kdeps.pop()
                while kdeps:
                    kz = kz + kdeps.pop()
                kz = kz * 0.0
                base = base + jnp.concatenate(
                    [jnp.concatenate([kz] * NC, axis=1)] * (DH // 8), axis=0)
            acc[uu] = base + a

        def gen_kb(hn, kb, d):
            t = bcast_key_column(kt_v[0, pl.ds(hn * DH + d, 1), :])
            kb[0, d] = t
            return t[KV - 8:KV]

        def link(uu, sb, c, start, e):
            zctr[0] += 1
            z = lax.shift_right_logical(i + zctr[0], 16)
            hh, qb = units[uu]
            kb = kbs[hh % 2][z, :, sb * SB:(sb + 1) * SB, :]
            qs = qb_v[qb * NC + c, pl.ds(head(uu) * (DH // 8) + z, DH // 8)]
            a = start
            for d in range(DH):
                q = qs[d // 8, d % 8]
                if e is not None and d == DH - 1:
                    q = q + e
                t = kb[d].reshape(SB // 8, 8, 128) * q[None]
                a = t if a is None else a + t
            return a

        def vpu_pv(uu, sb0, sb1):
            rows = [jnp.concatenate([pvp.pop((uu, sb, c)) for c in range(NC)], axis=1)
                    for sb in range(sb0, sb1)]
            pv(uu, sb0 * SB, (sb1 - sb0) * SB, jnp.concatenate(rows, axis=0))

        def fin(uu):
            l = lsum.pop(uu) + jnp.concatenate([lv.pop((uu, c)) for c in range(NC)], axis=1)
            ls = jnp.sum(l, axis=0, keepdims=True)
            a = acc.pop(uu)
            ok = jnp.logical_and(jnp.logical_and(ls >= L_LO, ls <= L_HI), jnp.abs(a) <= F32_BIG)
            bad[0] = jnp.where(ok, bad[0], 1.0)
            ot_v[hrows(head(uu)), qcols(uu)] = a * (1.0 / ls)

        for idx in range(n + 1):
            if idx < n:
                uu, kc = divmod(idx, NSL)
                if kc == 0:
                    wqs[uu] = masked_q(head(uu), qcols(uu))
                ss[idx] = jnp.dot(k_v[head(uu) // HPG, pl.ds(offs[kc], sizes[kc]), :], wqs[uu],
                                  preferred_element_type=F32)
            if idx >= 1:
                uu, kc = divmod(idx - 1, NSL)
                hh, qb = units[uu]
                p = jnp.exp2(ss.pop(idx - 1))
                r = fold(p, jnp.sum)
                lsum[uu] = r if kc == 0 else lsum[uu] + r
                pv(uu, offs[kc], sizes[kc], p, deadline=(idx - 1 == KBDL))
                hn = jnp.minimum(head(uu) + 1, H - 1)
                if hh == 0:
                    if kc < DH // NQ:
                        gen_kb(hn, kbs[1], qb * (DH // NQ) + kc)
                elif qb < DH // NSL:
                    kdeps.append(gen_kb(hn, kbs[0], qb * NSL + kc))
                lo = (kc * len(links)) // NSL
                hi = ((kc + 1) * len(links)) // NSL
                for li in range(lo, hi):
                    sb, c = links[li]
                    e = lagq.pop(0) if len(lagq) >= LAG else None
                    a = link(uu, sb, c, prev[0], e)
                    pe = jnp.exp2(a)
                    ls = jnp.sum(pe, axis=0)
                    key = (uu, c)
                    lv[key] = ls if key not in lv else lv[key] + ls
                    pvp[(uu, sb, c)] = pe.reshape(SB, 128)
                    prev[0] = a[0:1] * 0.0
                    lagq.append(jnp.minimum(lv[key], 0.0))
                if uu >= 1:
                    if kc == PVA:
                        vpu_pv(uu - 1, 0, NSB // 2)
                    if kc == PVB:
                        vpu_pv(uu - 1, NSB // 2, NSB)
                        fin(uu - 1)
        vpu_pv(NUU - 1, 0, NSB)
        fin(NUU - 1)
        return bad[0]

    bad = lax.fori_loop(0, H // HPB, fast_body, jnp.zeros((DH, TQ), F32))
    cp_modb.wait()

    def modulation(lo, hi):
        mod_v[:, lo * D:hi * D] = jnp.dot(sc_v[...].astype(BF16), wmod_v[:, lo * D:hi * D],
                                          preferred_element_type=F32)

    modulation(2, 3)

    @pl.when(jnp.max(bad) > 0.0)
    def _():
        def safe_body(u, carry):
            h = u // NQ
            cols = pl.ds(pl.multiple_of((u % NQ) * TQ, TQ), TQ)
            wq = masked_q(h, cols)
            acc = l = m = None
            for kc in range(S // KC):
                keys = pl.ds(kc * KC, KC)
                s = jnp.dot(k_v[h // HPG, keys, :], wq, preferred_element_type=F32)
                mc = jnp.max(fold(s, jnp.max), axis=0, keepdims=True)
                mn = mc if kc == 0 else jnp.maximum(m, mc)
                p = jnp.exp2(s - mn)
                a = jnp.dot(vt_v[hrows(h), keys], p.astype(BF16), preferred_element_type=F32)
                r = fold(p, jnp.sum)
                if kc == 0:
                    acc, l = a, r
                else:
                    al = jnp.exp2(m - mn)
                    acc, l = acc * al + a, l * al + r
                m = mn
            ot_v[hrows(h), cols] = acc * (1.0 / jnp.sum(l, axis=0, keepdims=True))
            return carry

        lax.fori_loop(0, H * NQ, safe_body, 0)

    cp_wo.wait()
    cp_win.wait()
    hbufs = (ha_v, hb_v)
    zbufs = (zga_v, zgb_v)

    def p3_a(i, hbuf, first=False):
        rows = _rows(i, TM)
        o = jnp.transpose(ot_v[:, rows]).astype(BF16)
        a = jnp.dot(o, wo_v[...], preferred_element_type=F32)
        if first:
            modulation(3, 6)
        x1 = x_v[rows, :].astype(F32) + modrow(2) * a
        x1_v[rows, :] = x1

        def emit(r0, y):
            hbuf[r0:r0 + LNP, :] = (y * (1.0 + modrow(4)) + modrow(3)).astype(BF16)

        if first:
            hbuf[...] = (_layernorm(x1) * (1.0 + modrow(4)) + modrow(3)).astype(BF16)
        else:
            _layernorm_pieces(lambda r0, n: x1[r0:r0 + n], TM, LNP, D, emit)

    def p3_block(i, t, z, with_next=True):
        h2 = hbufs[t][...]
        zbufs[t][0] = _gelu(jnp.dot(h2, win_v[:, FH:2 * FH], preferred_element_type=F32))
        if with_next:
            p3_a(i + 1, hbufs[1 - t])
        z1_v[_rows(i, TM), :] = jnp.dot(h2, win_v[:, 0:FH], preferred_element_type=F32)

        def emit(r0, y):
            z2_v[_rows(i, LNP, r0), :] = y.astype(BF16)

        _layernorm_pieces(lambda r0, n: zbufs[t][z, r0:r0 + n, :], TM, LNP, FH, emit)

    def p3_body(j, carry):
        for t in range(2):
            p3_block(j * 2 + t, t, lax.shift_right_logical(j, 16 + t))
        return carry

    p3_a(0, hbufs[0], first=True)
    zo = lax.fori_loop(0, NB // 2 - 1, p3_body, jnp.int32(0))
    p3_block(NB - 2, 0, zo)
    p3_block(NB - 1, 1, zo, with_next=False)

    cp_wsp.wait()
    cp_wout.wait()

    def out_copy(i):
        return pltpu.make_async_copy(obuf.at[_rows(i, TM), :], out_hbm.at[_rows(i, TM), :],
                                     osems.at[i])

    def p4_body(i, carry):
        rows = _rows(i, TM)
        g = jnp.dot(wsp_v[rows, :], z2_v[...], preferred_element_type=F32)
        g = g + jnp.concatenate([bcol_v[rows, :]] * (FH // 128), axis=1)
        t = (_gelu(z1_v[rows, :]) * g).astype(BF16)
        y = jnp.dot(t, wout_v[...], preferred_element_type=F32)
        obuf[rows, :] = (x1_v[rows, :] + modrow(5) * y).astype(BF16)
        out_copy(i).start()
        return carry

    lax.fori_loop(0, NB, p4_body, 0)
    for i in range(NB):
        out_copy(i).wait()


@jax.jit
def pallas_adaLN_cond__softmax_full_mha__mixer_gmlp__prompt_kernel(
    A_x: jax.Array,
    A_wqkv: jax.Array,
    A_wo: jax.Array,
    B_x: jax.Array,
    B_w_in: jax.Array,
    B_w_sp: jax.Array,
    B_b_sp: jax.Array,
    B_w_out: jax.Array,
    c: jax.Array,
    w_mod: jax.Array,
):
    B, S, D = A_x.shape
    F = B_w_in.shape[-1]
    FH = F // 2
    DH = D // H
    assert B == 1 and KV == TM
    any_spec = pl.BlockSpec(memory_space=pl.ANY)
    out = pl.pallas_call(
        functools.partial(_kernel, S=S, D=D, FH=FH),
        out_shape=jax.ShapeDtypeStruct((S, D), BF16),
        in_specs=[any_spec] * 9,
        out_specs=any_spec,
        scratch_shapes=[
            pltpu.VMEM((S, D), BF16),
            pltpu.VMEM((D, 3 * D), BF16),
            pltpu.VMEM((D, D), BF16),
            pltpu.VMEM((D, F), BF16),
            pltpu.VMEM((S, S), BF16),
            pltpu.VMEM((FH, D), BF16),
            pltpu.VMEM((D, 6 * D), BF16),
            pltpu.VMEM((H, 2, DH, D), BF16),
            pltpu.VMEM((8, 6 * D), F32),
            pltpu.VMEM((D // 128, S, 128), BF16),
            pltpu.VMEM((D, S), BF16),
            pltpu.VMEM((D, S), BF16),
            pltpu.VMEM((D, S), F32),
            pltpu.VMEM((S, D), F32),
            pltpu.VMEM((S, FH), F32),
            pltpu.VMEM((S, FH), BF16),
            pltpu.VMEM((S, 128), F32),
            pltpu.VMEM((S, D), BF16),
            pltpu.VMEM((2, TM, D), BF16),
            pltpu.VMEM((TM, D), BF16),
            pltpu.VMEM((TM, D), BF16),
            pltpu.VMEM((1, TM, FH), F32),
            pltpu.VMEM((1, TM, FH), F32),
            pltpu.VMEM((S // 128, D // 8, 8, 8, 128), F32),
            pltpu.VMEM((S // TM, D, TM), F32),
            pltpu.VMEM((1, DH, KV, 128), F32),
            pltpu.VMEM((1, DH, KV, 128), F32),
            pltpu.VMEM((S,), BF16),
            pltpu.VMEM((1, D), BF16),
            pltpu.VMEM((8, D), F32),
            pltpu.SemaphoreType.DMA((11,)),
            pltpu.SemaphoreType.DMA((S // TM,)),
            pltpu.SemaphoreType.DMA((S // TM,)),
        ],
        compiler_params=pltpu.CompilerParams(vmem_limit_bytes=112 * 1024 * 1024),
    )(A_x.reshape(S, D), A_wqkv, A_wo, B_w_in, B_w_sp, B_b_sp, B_w_out, c, w_mod)
    return out.reshape(B, S, D)
```

```python
import functools
import math

import jax
import jax.numpy as jnp
from jax import lax
import jax.experimental.pallas as pl
import jax.experimental.pallas.tpu as pltpu

F32 = jnp.float32
BF16 = jnp.bfloat16

H = 32
EPS = 1e-5
TM = 256
TQ = 512
KC = 256
KV = 256
SB = 32
HPB = 2
LAG = 2
PVA, PVB = 0, 2
KBDL = 48
LNP = 128
T4 = 512
TO = 128

L_LO = 2.0 ** -32
L_HI = 2.0 ** 64
F32_BIG = 3.0e38


def _layernorm(x):
    m = jnp.mean(x, axis=-1, keepdims=True)
    xc = x - m
    v = jnp.mean(xc * xc, axis=-1, keepdims=True)
    return xc * lax.rsqrt(v + EPS)


def _layernorm_pieces(load, nrows, piece, width, emit):
    dep = None
    for r0 in range(0, nrows, piece):
        x = load(r0, piece)
        s = x[:, 0:128] if dep is None else x[:, 0:128] + dep
        for c in range(1, width // 128):
            s = s + x[:, c * 128:(c + 1) * 128]
        m = jnp.sum(s, axis=-1, keepdims=True) * (1.0 / width)
        xc = x - m
        sq = xc * xc
        v = sq[:, 0:128]
        for c in range(1, width // 128):
            v = v + sq[:, c * 128:(c + 1) * 128]
        v = jnp.sum(v, axis=-1, keepdims=True) * (1.0 / width)
        y = xc * lax.rsqrt(v + EPS)
        emit(r0, y)
        dep = y[:, width - 128:width] * 0.0


def _gelu(x):
    c = math.sqrt(2.0 / math.pi)
    return 0.5 * x * (1.0 + jnp.tanh(x * (c + (c * 0.044715) * (x * x))))


def _rows(i, n, off=0):
    if isinstance(i, int):
        return pl.ds(i * TM + off, n)
    return pl.ds(pl.multiple_of(i * TM + off, math.gcd(TM, off)), n)


def _kernel(x_hbm, wqkv_hbm, wo_hbm, win_hbm, wsp_hbm, bsp_hbm, wout_hbm, c_hbm, wmod_hbm,
            out_hbm,
            x_v, wqkv_v, wo_v, win_v, wsp_v, wout_v, wmod_v,
            wqvt_v, mod_v, k_v, qt_v, vt_v, ot_v, x1_v, z1_v, z2_v, bcol_v, obuf,
            h1_v, ha_v, hb_v, zga_v, zgb_v, qb_v, kt_v, kb0, kb1, pre_v, lpre_v, bsp_v, c_v, sc_v,
            sems, xsems, osems, *, S, D, FH):
    DH = D // H
    NQ = S // TQ
    NB = S // TM
    HPG = 128 // DH
    NC = TQ // 128

    def cp(src, dst, n):
        return pltpu.make_async_copy(src, dst, sems.at[n])

    def cp_x(i):
        return pltpu.make_async_copy(x_hbm.at[_rows(i, TM), :], x_v.at[_rows(i, TM), :],
                                     xsems.at[i])

    cp_c = cp(c_hbm, c_v, 0)
    cp_b = cp(bsp_hbm, bsp_v, 1)
    cp_moda = cp(wmod_hbm.at[:, 0:2 * D], wmod_v.at[:, 0:2 * D], 2)
    cp_wq = cp(wqkv_hbm.at[:, 0:D], wqkv_v.at[:, 0:D], 3)
    cp_wv = cp(wqkv_hbm.at[:, 2 * D:3 * D], wqkv_v.at[:, 2 * D:3 * D], 4)
    cp_wk = cp(wqkv_hbm.at[:, D:2 * D], wqkv_v.at[:, D:2 * D], 5)
    cp_modb = cp(wmod_hbm.at[:, 2 * D:6 * D], wmod_v.at[:, 2 * D:6 * D], 6)
    cp_wo = cp(wo_hbm, wo_v, 7)
    cp_win = cp(win_hbm, win_v, 8)
    cp_wsp = cp(wsp_hbm, wsp_v, 9)
    cp_wout = cp(wout_hbm, wout_v, 10)

    cp_b.start()
    cp_c.start()
    cp_x(0).start()
    cp_moda.start()
    cp_b.wait()
    bcol_v[...] = jnp.transpose(
        jnp.broadcast_to(bsp_v[...].astype(F32).reshape(1, S), (128, S)))
    cp_c.wait()
    cf = c_v[...].astype(F32)
    sc_v[...] = jnp.broadcast_to(cf * (1.0 / (1.0 + jnp.exp(-cf))), (8, D))
    cp_x(0).wait()
    cp_wk.start()
    xn0 = _layernorm(x_v[0:TM, :].astype(F32))
    cp_moda.wait()
    cp_wq.start()
    cp_wv.start()
    mod_v[:, 0:2 * D] = jnp.dot(sc_v[...].astype(BF16), wmod_v[:, 0:2 * D],
                                preferred_element_type=F32)

    def modrow(i):
        return mod_v[0:1, i * D:(i + 1) * D]

    def affine1(xn):
        return (xn * (1.0 + modrow(1)) + modrow(0)).astype(BF16)

    qscale = (DH ** -0.5) * math.log2(math.e)

    def bcast_key_column(row):
        return jnp.transpose(jnp.broadcast_to(row, (128, KV)))

    def p1_k(i, h):
        k32 = jnp.dot(h, wqkv_v[:, D:2 * D], preferred_element_type=F32)
        k = k32.astype(BF16)
        for g in range(D // 128):
            k_v[g, _rows(i, TM), :] = k[:, g * 128:(g + 1) * 128]
        return k32

    def p1_qv(i, h):
        for t in range(DH // NB):
            d = i * (DH // NB) + t
            kb0[0, d] = bcast_key_column(kt_v[pl.ds(d, 1), :])
        for c in range(TM // 128):
            cols = _rows(i, 128, c * 128)
            qvt = lax.dot_general(wqvt_v[...].reshape(2 * D, D), h[c * 128:(c + 1) * 128],
                                  (((1,), (1,)), ((), ())), preferred_element_type=F32)
            qvt = qvt.reshape(H, 2, DH, 128)
            q32 = qvt[:, 0].reshape(D, 128) * qscale
            qt_v[:, cols] = q32.astype(BF16)
            vt_v[:, cols] = qvt[:, 1].reshape(D, 128).astype(BF16)
            q3 = q32.reshape(D // 8, 8, 128)
            for r in range(8):
                qb_v[i * (TM // 128) + c, :, r] = jnp.broadcast_to(q3[:, r:r + 1, :],
                                                                   (D // 8, 8, 128))

    h0 = affine1(xn0)
    h1_v[0] = h0
    cp_wk.wait()
    cp_x(1).start()
    kt_v[...] = jnp.transpose(p1_k(0, h0))
    cp_wq.wait()
    cp_x(2).start()
    wqvt_v[:, 0] = jnp.transpose(wqkv_v[:, 0:D].astype(F32)).astype(BF16).reshape(H, DH, D)
    cp_wv.wait()
    for i in range(3, NB):
        cp_x(i).start()
    cp_modb.start()
    wqvt_v[:, 1] = jnp.transpose(
        wqkv_v[:, 2 * D:3 * D].astype(F32)).astype(BF16).reshape(H, DH, D)

    def p1_body(i, carry):
        cp_x(i + 1).wait()
        h = h1_v[i % 2]
        hn = affine1(_layernorm(x_v[_rows(i + 1, TM), :].astype(F32)))
        p1_qv(i, h)
        h1_v[(i + 1) % 2] = hn
        p1_k(i + 1, hn)
        return carry

    lax.fori_loop(0, NB - 1, p1_body, 0)
    p1_qv(NB - 1, h1_v[(NB - 1) % 2])
    for c_ in (cp_wo, cp_win, cp_wsp, cp_wout):
        c_.start()

    NSB = KV // SB
    sizes = [KC] * (S // KC)
    sizes[PVA] = KC // 2
    sizes[PVB] = KC // 2
    offs = [KV + sum(sizes[:c]) for c in range(len(sizes))]
    NSL = len(sizes)
    kbs = (kb0, kb1)

    def hrows(h):
        if isinstance(h, int):
            return pl.ds(h * DH, DH)
        return pl.ds(pl.multiple_of(h * DH, DH), DH)

    def masked_q(h, cols):
        q = qt_v[hrows(h), cols]
        qrep = jnp.concatenate([q] * HPG, axis=0)
        rows = lax.broadcasted_iota(jnp.int32, (128, TQ), 0)
        return jnp.where((rows // DH) == (h % HPG), qrep, jnp.zeros_like(qrep))

    def fold(x, op):
        return op(x.reshape(x.shape[0] // 8, 8, TQ), axis=0)

    def first_scores(h):
        wq = masked_q(h, pl.ds(0, TQ))
        return jnp.dot(k_v[h // HPG, pl.ds(offs[0], sizes[0]), :], wq,
                       preferred_element_type=F32)

    def store_first(s_):
        p = jnp.exp2(s_)
        pre_v[0:KC // 2, :] = p.astype(BF16)
        lpre_v[...] = fold(p, jnp.sum)

    store_first(first_scores(0))

    def fast_body(i, bad0):
        units = [(hh, qb) for hh in range(HPB) for qb in range(NQ)]
        NUU = len(units)
        n = NUU * NSL
        wqs, ss, acc, lsum, lv, pvp = {}, {}, {}, {}, {}, {}
        prev = [None]
        lagq, kdeps = [], []
        bad = [bad0]
        links = [(sb, c) for sb in range(NSB) for c in range(NC)]
        zctr = [0]

        def head(uu):
            return i * HPB + units[uu][0]

        def qcols(uu):
            return pl.ds(units[uu][1] * TQ, TQ)

        def pv(uu, off, n_, p, deadline=False):
            a = jnp.dot(vt_v[hrows(head(uu)), pl.ds(off, n_)], p.astype(BF16),
                        preferred_element_type=F32)
            base = acc[uu] if uu in acc else bad[0] * 0.0
            if deadline:
                kz = kdeps.pop()
                while kdeps:
                    kz = kz + kdeps.pop()
                kz = kz * 0.0
                base = base + jnp.concatenate(
                    [jnp.concatenate([kz] * NC, axis=1)] * (DH // 8), axis=0)
            acc[uu] = base + a

        def gen_kb(hn, kb, d):
            t = bcast_key_column(kt_v[pl.ds(hn * DH + d, 1), :])
            kb[0, d] = t
            return t[KV - 8:KV]

        def link(uu, sb, c, start, e):
            zctr[0] += 1
            z = lax.shift_right_logical(i + zctr[0], 16)
            hh, qb = units[uu]
            kb = kbs[hh % 2][z, :, sb * SB:(sb + 1) * SB, :]
            qs = qb_v[qb * NC + c, pl.ds(head(uu) * (DH // 8) + z, DH // 8)]
            a = start
            for d in range(DH):
                q = qs[d // 8, d % 8]
                if e is not None and d == DH - 1:
                    q = q + e
                t = kb[d].reshape(SB // 8, 8, 128) * q[None]
                a = t if a is None else a + t
            return a

        def vpu_pv(uu, sb0, sb1):
            rows = [jnp.concatenate([pvp.pop((uu, sb, c)) for c in range(NC)], axis=1)
                    for sb in range(sb0, sb1)]
            pv(uu, sb0 * SB, (sb1 - sb0) * SB, jnp.concatenate(rows, axis=0))

        def fin(uu):
            l = lsum.pop(uu) + jnp.concatenate([lv.pop((uu, c)) for c in range(NC)], axis=1)
            ls = jnp.sum(l, axis=0, keepdims=True)
            a = acc.pop(uu)
            ok = jnp.logical_and(jnp.logical_and(ls >= L_LO, ls <= L_HI), jnp.abs(a) <= F32_BIG)
            bad[0] = jnp.where(ok, bad[0], 1.0)
            ot_v[hrows(head(uu)), qcols(uu)] = a * (1.0 / ls)

        hnext = jnp.minimum(i * HPB + HPB, H - 1)
        for idx in range(1, n + 1):
            if idx < n:
                uu, kc = divmod(idx, NSL)
                if uu not in wqs:
                    wqs[uu] = masked_q(head(uu), qcols(uu))
                ss[idx] = jnp.dot(k_v[head(uu) // HPG, pl.ds(offs[kc], sizes[kc]), :], wqs[uu],
                                  preferred_element_type=F32)
            else:
                ahead = first_scores(hnext)
            uu, kc = divmod(idx - 1, NSL)
            hh, qb = units[uu]
            if uu >= 1:
                if kc == PVA:
                    vpu_pv(uu - 1, 0, NSB // 2)
                if kc == PVB:
                    vpu_pv(uu - 1, NSB // 2, NSB)
                    fin(uu - 1)
            if idx == 1:
                p = pre_v[0:KC // 2, :]
                lsum[uu] = lpre_v[...]
            else:
                p = jnp.exp2(ss.pop(idx - 1))
                r = fold(p, jnp.sum)
                lsum[uu] = r if kc == 0 else lsum[uu] + r
            pv(uu, offs[kc], sizes[kc], p, deadline=(idx - 1 == KBDL))
            hn = jnp.minimum(head(uu) + 1, H - 1)
            if hh == 0:
                if kc < DH // NQ:
                    gen_kb(hn, kbs[1], qb * (DH // NQ) + kc)
            elif qb < DH // NSL:
                kdeps.append(gen_kb(hn, kbs[0], qb * NSL + kc))
            lo = (kc * len(links)) // NSL
            hi = ((kc + 1) * len(links)) // NSL
            for li in range(lo, hi):
                sb, c = links[li]
                e = lagq.pop(0) if len(lagq) >= LAG else None
                a = link(uu, sb, c, prev[0], e)
                pe = jnp.exp2(a)
                ls = jnp.sum(pe, axis=0)
                key = (uu, c)
                lv[key] = ls if key not in lv else lv[key] + ls
                pvp[(uu, sb, c)] = pe.reshape(SB, 128)
                prev[0] = a[0:1] * 0.0
                lagq.append(jnp.minimum(lv[key], 0.0))
        vpu_pv(NUU - 1, 0, NSB)
        fin(NUU - 1)
        store_first(ahead)
        return bad[0]

    bad = lax.fori_loop(0, H // HPB, fast_body, jnp.zeros((DH, TQ), F32))
    cp_modb.wait()

    def modulation(lo, hi):
        mod_v[:, lo * D:hi * D] = jnp.dot(sc_v[...].astype(BF16), wmod_v[:, lo * D:hi * D],
                                          preferred_element_type=F32)

    modulation(2, 3)

    @pl.when(jnp.max(bad) > 0.0)
    def _():
        def safe_body(u, carry):
            h = u // NQ
            cols = pl.ds(pl.multiple_of((u % NQ) * TQ, TQ), TQ)
            wq = masked_q(h, cols)
            acc = l = m = None
            for kc in range(S // KC):
                keys = pl.ds(kc * KC, KC)
                s = jnp.dot(k_v[h // HPG, keys, :], wq, preferred_element_type=F32)
                mc = jnp.max(fold(s, jnp.max), axis=0, keepdims=True)
                mn = mc if kc == 0 else jnp.maximum(m, mc)
                p = jnp.exp2(s - mn)
                a = jnp.dot(vt_v[hrows(h), keys], p.astype(BF16), preferred_element_type=F32)
                r = fold(p, jnp.sum)
                if kc == 0:
                    acc, l = a, r
                else:
                    al = jnp.exp2(m - mn)
                    acc, l = acc * al + a, l * al + r
                m = mn
            ot_v[hrows(h), cols] = acc * (1.0 / jnp.sum(l, axis=0, keepdims=True))
            return carry

        lax.fori_loop(0, H * NQ, safe_body, 0)

    cp_wo.wait()
    cp_win.wait()
    hbufs = (ha_v, hb_v)
    zbufs = (zga_v, zgb_v)

    def p3_a(i, hbuf, first=False):
        rows = _rows(i, TM)
        o = jnp.transpose(ot_v[:, rows]).astype(BF16)
        a = jnp.dot(o, wo_v[...], preferred_element_type=F32)
        if first:
            modulation(3, 6)
        x1 = x_v[rows, :].astype(F32) + modrow(2) * a
        x1_v[rows, :] = x1

        def emit(r0, y):
            hbuf[r0:r0 + LNP, :] = (y * (1.0 + modrow(4)) + modrow(3)).astype(BF16)

        if first:
            hbuf[...] = (_layernorm(x1) * (1.0 + modrow(4)) + modrow(3)).astype(BF16)
        else:
            _layernorm_pieces(lambda r0, n: x1[r0:r0 + n], TM, LNP, D, emit)

    def p3_block(i, t, z, with_next=True):
        h2 = hbufs[t][...]
        zbufs[t][0] = _gelu(jnp.dot(h2, win_v[:, FH:2 * FH], preferred_element_type=F32))
        if with_next:
            p3_a(i + 1, hbufs[1 - t])
        z1_v[_rows(i, TM), :] = jnp.dot(h2, win_v[:, 0:FH], preferred_element_type=F32)

        def emit(r0, y):
            z2_v[_rows(i, LNP, r0), :] = y.astype(BF16)

        _layernorm_pieces(lambda r0, n: zbufs[t][z, r0:r0 + n, :], TM, LNP, FH, emit)

    def p3_body(j, carry):
        for t in range(2):
            p3_block(j * 2 + t, t, lax.shift_right_logical(j, 16 + t))
        return carry

    p3_a(0, hbufs[0], first=True)
    zo = lax.fori_loop(0, NB // 2 - 1, p3_body, jnp.int32(0))
    p3_block(NB - 2, 0, zo)
    p3_block(NB - 1, 1, zo, with_next=False)

    cp_wsp.wait()
    cp_wout.wait()

    def rows4(i, off=0, n=T4):
        if isinstance(i, int):
            return pl.ds(i * T4 + off, n)
        return pl.ds(pl.multiple_of(i * T4 + off, TO), n)

    def out_copy(i, t):
        r = rows4(i, t * TO, TO)
        return pltpu.make_async_copy(obuf.at[r, :], out_hbm.at[r, :],
                                     osems.at[i * (T4 // TO) + t])

    def p4_body(i, carry):
        rows = rows4(i)
        g = jnp.dot(wsp_v[rows, :], z2_v[...], preferred_element_type=F32)
        g = g + jnp.concatenate([bcol_v[rows, :]] * (FH // 128), axis=1)
        t_ = (_gelu(z1_v[rows, :]) * g).astype(BF16)
        for t in range(T4 // TO):
            r = rows4(i, t * TO, TO)
            y = jnp.dot(t_[t * TO:(t + 1) * TO], wout_v[...], preferred_element_type=F32)
            obuf[r, :] = (x1_v[r, :] + modrow(5) * y).astype(BF16)
            out_copy(i, t).start()
        return carry

    lax.fori_loop(0, S // T4, p4_body, 0)
    for i in range(S // T4):
        for t in range(T4 // TO):
            out_copy(i, t).wait()


@jax.jit
def pallas_adaLN_cond__softmax_full_mha__mixer_gmlp__prompt_kernel(
    A_x: jax.Array,
    A_wqkv: jax.Array,
    A_wo: jax.Array,
    B_x: jax.Array,
    B_w_in: jax.Array,
    B_w_sp: jax.Array,
    B_b_sp: jax.Array,
    B_w_out: jax.Array,
    c: jax.Array,
    w_mod: jax.Array,
):
    B, S, D = A_x.shape
    F = B_w_in.shape[-1]
    FH = F // 2
    DH = D // H
    assert B == 1 and KV == TM
    any_spec = pl.BlockSpec(memory_space=pl.ANY)
    out = pl.pallas_call(
        functools.partial(_kernel, S=S, D=D, FH=FH),
        out_shape=jax.ShapeDtypeStruct((S, D), BF16),
        in_specs=[any_spec] * 9,
        out_specs=any_spec,
        scratch_shapes=[
            pltpu.VMEM((S, D), BF16),
            pltpu.VMEM((D, 3 * D), BF16),
            pltpu.VMEM((D, D), BF16),
            pltpu.VMEM((D, F), BF16),
            pltpu.VMEM((S, S), BF16),
            pltpu.VMEM((FH, D), BF16),
            pltpu.VMEM((D, 6 * D), BF16),
            pltpu.VMEM((H, 2, DH, D), BF16),
            pltpu.VMEM((8, 6 * D), F32),
            pltpu.VMEM((D // 128, S, 128), BF16),
            pltpu.VMEM((D, S), BF16),
            pltpu.VMEM((D, S), BF16),
            pltpu.VMEM((D, S), F32),
            pltpu.VMEM((S, D), F32),
            pltpu.VMEM((S, FH), F32),
            pltpu.VMEM((S, FH), BF16),
            pltpu.VMEM((S, 128), F32),
            pltpu.VMEM((S, D), BF16),
            pltpu.VMEM((2, TM, D), BF16),
            pltpu.VMEM((TM, D), BF16),
            pltpu.VMEM((TM, D), BF16),
            pltpu.VMEM((1, TM, FH), F32),
            pltpu.VMEM((1, TM, FH), F32),
            pltpu.VMEM((S // 128, D // 8, 8, 8, 128), F32),
            pltpu.VMEM((D, KV), F32),
            pltpu.VMEM((1, DH, KV, 128), F32),
            pltpu.VMEM((1, DH, KV, 128), F32),
            pltpu.VMEM((KC // 2, TQ), BF16),
            pltpu.VMEM((8, TQ), F32),
            pltpu.VMEM((S,), BF16),
            pltpu.VMEM((1, D), BF16),
            pltpu.VMEM((8, D), F32),
            pltpu.SemaphoreType.DMA((11,)),
            pltpu.SemaphoreType.DMA((S // TM,)),
            pltpu.SemaphoreType.DMA((S // TO,)),
        ],
        compiler_params=pltpu.CompilerParams(vmem_limit_bytes=112 * 1024 * 1024),
    )(A_x.reshape(S, D), A_wqkv, A_wo, B_w_in, B_w_sp, B_b_sp, B_w_out, c, w_mod)
    return out.reshape(B, S, D)
```
